```python
import jax
import jax.numpy as jnp

def _softmax(x, axis=-1):
    return jax.nn.softmax(x, axis=axis)

def _gelu(x):
    return jax.nn.gelu(x, approximate=True)

def _silu(x):
    return jax.nn.silu(x)

def _sigmoid(x):
    return jax.nn.sigmoid(x)

def _layernorm(x, axis=-1, eps=1e-05):
    m = jnp.mean(x, axis=axis, keepdims=True)
    v = jnp.var(x, axis=axis, keepdims=True)
    return (x - m) / jnp.sqrt(v + eps)

def _scatter_add(tgt, idx, src, axis=0):
    return tgt.at[idx].add(src)

def _segment_sum(src, seg, n):
    return jax.ops.segment_sum(src, seg, n)

class _Rng:

    def __init__(self, key):
        self._k = key

    def _next(self):
        self._k, sub = jax.random.split(self._k)
        return sub

    def normal(self, shape):
        return jax.random.normal(self._next(), shape, dtype=jnp.bfloat16)

    def randint(self, lo, hi, shape):
        return jax.random.randint(self._next(), shape, lo, hi, dtype=jnp.int32)

    def uniform(self, shape, lo=0.0, hi=1.0):
        return jax.random.uniform(self._next(), shape, jnp.bfloat16, lo, hi)

    def permutation(self, n):
        return jax.random.permutation(self._next(), n)
kernel_name = 'adaLN_cond__sliding_block_cached__dense_activation_mish__decode'

def setup_inputs():
    _rng = _Rng(jax.random.key(int.from_bytes(__import__("os").urandom(4), "little")))
    _w = lambda a: (lambda t: t.astype(jnp.bfloat16) if jnp.issubdtype(t.dtype, jnp.floating) else t)(jnp.asarray(a))

    def _A_setup():
        B, Sq, D = (1, 1, 640)
        Hq, Hkv, Sk, Dh = (32, 32, 32768, 192)
        assert Hq % Hkv == 0, (Hq, Hkv)
        return {'x': _w((lambda *s: _rng.normal(s) * 0.05)(B, Sq, D)), 'k_cache': _w((lambda *s: _rng.normal(s) * 0.05)(B, Hkv, Sk, Dh)), 'v_cache': _w((lambda *s: _rng.normal(s) * 0.05)(B, Hkv, Sk, Dh)), 'wq': _w((lambda *s: _rng.normal(s) * 0.05)(D, Hq * Dh) * D ** (-0.5)), 'wo': _w((lambda *s: _rng.normal(s) * 0.05)(Hq * Dh, D) * (Hq * Dh) ** (-0.5))}
    _A_in = _A_setup()

    def _B_setup():
        B, S, D, F = (1, 1, 640, 1536)
        return {'x': _w((lambda *s: _rng.normal(s) * 0.05)(B, S, D)), 'w1': _w((lambda *s: _rng.normal(s) * 0.05)(D, F) * D ** (-0.5)), 'b1': _w((lambda *s: _rng.normal(s) * 0.05)(F)), 'w2': _w((lambda *s: _rng.normal(s) * 0.05)(F, D) * F ** (-0.5))}
    _B_in = _B_setup()
    return {'A_x': _A_in['x'], 'A_k_cache': _A_in['k_cache'], 'A_v_cache': _A_in['v_cache'], 'A_wq': _A_in['wq'], 'A_wo': _A_in['wo'], 'B_x': _B_in['x'], 'B_w1': _B_in['w1'], 'B_b1': _B_in['b1'], 'B_w2': _B_in['w2'], 'c': _w((lambda *s: _rng.normal(s) * 0.05)(1, 640)), 'w_mod': _w((lambda *s: _rng.normal(s) * 0.05)(640, 6 * 640) * 640 ** (-0.5))}

def reference(A_x, A_k_cache, A_v_cache, A_wq, A_wo, B_x, B_w1, B_b1, B_w2, c, w_mod):

    def _A_ref(x, k_cache, v_cache, wq, wo):
        B, Sq, D = x.shape
        Hq, Dh = (32, 192)
        Hkv, Sk = (k_cache.shape[1], k_cache.shape[2])
        W = min(4096, max(256, Sk // 4))
        rep = Hq // Hkv
        q = (lambda x, *d: x.transpose(*d))((x @ wq).reshape(B, Sq, Hq, Dh), 0, 2, 1, 3)
        k = jnp.repeat(k_cache[:, :, Sk - W:, :], rep, axis=1)
        v = jnp.repeat(v_cache[:, :, Sk - W:, :], rep, axis=1)
        scores = jnp.einsum('bhqd,bhkd->bhqk', q, k) * Dh ** (-0.5)
        p = _softmax(scores, axis=-1)
        o = jnp.einsum('bhqk,bhkd->bhqd', p, v)
        return (lambda x, *d: x.transpose(*d))(o, 0, 2, 1, 3).reshape(B, Sq, Hq * Dh) @ wo

    def _B_ref(x, w1, b1, w2):
        h = jnp.einsum('bsd,df->bsf', x, w1) + b1
        sp = jnp.log1p(jnp.exp(-jnp.abs(h))) + jnp.where(h > 0, h, jnp.zeros_like(h))
        act = h * jnp.tanh(sp)
        return jnp.einsum('bsf,fd->bsd', act, w2)
    x = A_x
    mod = (_silu(c) @ w_mod).reshape(c.shape[0], 6, 1, -1)
    sa, ca, ga, sb, cb, gb = (mod[:, 0].copy(), mod[:, 1].copy(), mod[:, 2].copy(), mod[:, 3].copy(), mod[:, 4].copy(), mod[:, 5].copy())
    h = _layernorm(x, axis=-1) * (1 + ca) + sa
    x = x + ga * _A_ref(h, A_k_cache, A_v_cache, A_wq, A_wo)
    h = _layernorm(x, axis=-1) * (1 + cb) + sb
    x = x + gb * _B_ref(h, B_w1, B_b1, B_w2)
    return x
```

```python
import functools

import jax
import jax.numpy as jnp
from jax import lax
import jax.experimental.pallas as pl
import jax.experimental.pallas.tpu as pltpu

D = 640
H = 32
DH = 192
F = 1536
PAIR = 2 * DH
NPAIR = H // 2
SUB, LANE = 8, 128
WIDE = D // LANE
F32 = jnp.float32
BF16 = jnp.bfloat16

NSLOT = 3
SKEW = 25
LOOK = 22
KV_COPY = (4,) * 6, 4
V_LAST_COPY = (4,) * 12, 4
WQ_COPY = WO_COPY = (3,) * 5, 4
WMOD_COPY = (2,) * 3, 8
W1_COPY = W2_COPY = (2,) * 2, 8
W2_END_COPY = (1,) * 4, 2
V_LAST_PARTS = (2048, 3072, 4096)
W2_PARTS = (160, 208, 226, 240)
STEP = 512


def _layernorm(x, eps=1e-5):
    m = jnp.mean(x, axis=-1, keepdims=True)
    d = x - m
    v = jnp.mean(d * d, axis=-1, keepdims=True)
    return d / jnp.sqrt(v + eps)


def _mish(u):
    softplus = jnp.log1p(jnp.exp(-jnp.abs(u))) + jnp.where(u > 0, u, 0.0)
    return u * jnp.tanh(softplus)


def _dot(a, b):
    return jnp.dot(a, b, preferred_element_type=F32)


def _tiles(w, places):
    r, c = w.shape
    return w.reshape(r // SUB, SUB, c // LANE, LANE).transpose(0, 2, 1, 3).reshape(places, -1, LANE)


def _view(ref, n):
    return ref.reshape(n, ref.shape[0] // n, LANE)


def _columns(ref, start, n):
    cols = []
    for c in range(0, n, 2):
        two = ref[:, pl.ds(start + SUB * c, 2 * SUB), :]
        cols += [two[:, :SUB].reshape(-1, LANE), two[:, SUB:].reshape(-1, LANE)]
    return jnp.concatenate(cols, axis=1)


def _narrow(tiles):
    w = tiles.reshape(-1, 2 * SUB * WIDE, LANE)
    cols = [jnp.concatenate([w[:, SUB * c:SUB * (c + 1)], w[:, SUB * (c + WIDE):SUB * (c + WIDE + 1)]], axis=1)
            for c in range(WIDE)]
    return jnp.concatenate([c.reshape(-1, LANE) for c in cols], axis=1)


def _sweeps(src, dst, rows, how, tag, sem, src_at=(0, 0), dst_at=(0, 0)):
    places, tiles = how
    out = []
    for t in range(0, rows, SUB * tiles):
        w = min(SUB * tiles, rows - t)
        s, sweep = 0, []
        for n in places:
            sweep.append((tag, functools.partial(
                pltpu.make_async_copy, src.at[pl.ds(src_at[0] + s, n), pl.ds(src_at[1] + t, w)],
                dst.at[pl.ds(dst_at[0] + s, n), pl.ds(dst_at[1] + t, w)], sem)))
            s += n
        out.append(sweep)
    return out


def _chain(*lists):
    keyed = [((i + 0.5) / len(l), k, x) for k, l in enumerate(lists) for i, x in enumerate(l)]
    return [cp for _, _, sweep in sorted(keyed, key=lambda t: t[:2]) for cp in sweep]


class _Stream:
    def __init__(self, copies, started=(0, 0), end=()):
        self.queue = (copies[0::2], copies[1::2] + list(end))
        self.last = {tag: i // 2 for i, (tag, _) in enumerate(copies)}
        self.started = list(started)

    def start(self, q, n=1):
        for _, copy in self.queue[q][self.started[q]:self.started[q] + n]:
            copy().start(priority=q)
            self.started[q] += 1

    def more(self, n):
        for _ in range(n):
            self.start(1)
            self.start(0)

    def upto(self, n):
        self.more(n - self.started[0])

    def wait(self, tag, ref, sem):
        self.upto(self.last.get(tag, len(self.queue[0])) + 1 + LOOK)
        assert all(t != tag for q in range(2) for t, _ in self.queue[q][self.started[q]:])
        _wait_all(ref, sem)


def _wait_all(ref, sem):
    pltpu.make_async_copy(ref, ref, sem).wait()


def _kernel(x_hbm, k_hbm, v_hbm, wq_hbm, wo_hbm, w1_hbm, b1_hbm, w2_hbm, c_hbm, wmod_hbm, o_ref,
            buf, x_v, c_v, b1_v, q_s, s_s, att_s, mod_s, act_s, sem_w, sem_kv, sem_v, sem_w2, *, window):
    rows = window // LANE * SUB
    regions, n = [], 0
    for size in (2 * NSLOT * PAIR * window, D * H * DH, H * DH * D, 6 * D * D, D * F, F * D):
        regions.append(buf.at[pl.ds(n, size // LANE)])
        n += size // LANE
    kv_v, wq_v, wo_v, wmod_v, w1_v, w2_v = regions
    kv_v = _view(kv_v, PAIR // SUB)

    def kv_at(slot, j):
        at = (2 * slot + j) * rows
        return at if isinstance(at, int) else pl.multiple_of(at, rows)

    def kv_copies(p, slot, j, how, tag, sem, part=(0, window)):
        src = (k_hbm, v_hbm)[j]
        t0, t1 = (c // LANE * SUB for c in part)
        return [cp for r in range(0, PAIR // SUB, sum(how[0]))
                for cp in _chain(_sweeps(src, kv_v, t1 - t0, how, tag, sem,
                                         (p * (PAIR // SUB) + r, src.shape[1] - rows + t0), (r, kv_at(slot, j) + t0)))]

    def pair_copies(p, slot):
        return [cp for j in range(2) for cp in kv_copies(p, slot, j, KV_COPY, "kv", sem_kv.at[slot, j])]

    def weights(src, dst, how, i):
        return _sweeps(src, _view(dst, src.shape[0]), src.shape[1], how, i, sem_w.at[i])

    s_c, s_x, s_b1, s_wmod, s_wq, s_wo, s_w1 = range(7)
    small = [functools.partial(pltpu.make_async_copy, s, d, sem_w.at[i])
             for i, s, d in ((s_c, c_hbm, c_v), (s_x, x_hbm, x_v), (s_b1, b1_hbm, b1_v))]
    per_pair = len(pair_copies(0, 0)) // 2
    lead = LOOK + SKEW
    assert 2 * lead <= per_pair

    head = _Stream(_chain(weights(wq_hbm, wq_v, WQ_COPY, s_wq), weights(wmod_hbm, wmod_v, WMOD_COPY, s_wmod))
                   + _chain(weights(wo_hbm, wo_v, WO_COPY, s_wo), weights(w1_hbm, w1_v, W1_COPY, s_w1))
                   + pair_copies(0, 0) + pair_copies(1, 1)[:2 * lead])
    head.start(0)
    head.start(1, SKEW + 1)
    for cp in small:
        cp().start()
    head.wait(s_wmod, wmod_v, sem_w.at[s_wmod])
    head.wait(s_wq, wq_v, sem_w.at[s_wq])
    for cp in small:
        cp().wait()
    cf = c_v[...].astype(F32)
    silu_c = jnp.broadcast_to(cf * jax.nn.sigmoid(cf), (SUB, D)).astype(BF16)
    for i in range(0, 6 * WIDE, 2):
        mod_s[:, i * LANE:(i + 2) * LANE] = _dot(silu_c, _columns(_view(wmod_v, D // SUB), SUB * i, 2))
        head.more(2)

    def mod(i):
        return mod_s[:, i * D:(i + 1) * D]

    x0 = jnp.broadcast_to(x_v[...].astype(F32), (SUB, D))
    h = (_layernorm(x0) * (1.0 + mod(1)) + mod(0)).astype(BF16)
    row = lax.broadcasted_iota(jnp.int32, (SUB, PAIR), 0)
    col = lax.broadcasted_iota(jnp.int32, (SUB, PAIR), 1)
    own = jnp.logical_or(jnp.logical_and(row == 0, col < DH), jnp.logical_and(row == 1, col >= DH))
    for i in range(0, H * DH // LANE, 2):
        q = _dot(h, _columns(_view(wq_v, D // SUB), SUB * i, 2))
        for u in range(2):
            p, j = divmod(i + u, PAIR // LANE)
            q_s[p, :, j * LANE:(j + 1) * LANE] = jnp.where(
                own[:, j * LANE:(j + 1) * LANE], q[:, u * LANE:(u + 1) * LANE], 0.0)
        head.more(2)
    att_s[...] = jnp.zeros(att_s.shape, F32)
    head.upto(len(head.queue[0]) - SKEW)
    _wait_all(wo_v, sem_w.at[s_wo])
    _wait_all(w1_v, sem_w.at[s_w1])

    def kv_part(slot, j, c0=0, c1=window):
        return kv_v.at[:, pl.ds(kv_at(slot, j) + c0 // LANE * SUB, (c1 - c0) // LANE * SUB)]

    def kv_step(slot, j, c):
        return _columns(kv_v, kv_at(slot, j) + c // LANE * SUB, STEP // LANE)

    def softmax(p, slot, stream, pace):
        q = q_s[p].astype(BF16)
        for c in range(0, window, STEP):
            s_s[:, c:c + STEP] = _dot(q, kv_step(slot, 0, c)) * DH ** -0.5
            stream.more(pace)
        s = s_s[...]
        e = jnp.exp(s - jnp.max(s, axis=-1, keepdims=True))
        s_s[...] = e
        return jnp.sum(e, axis=-1, keepdims=True)

    def add_values(acc, slot, c0, c1, stream, pace):
        for c in range(c0, c1, STEP):
            acc += lax.dot_general(s_s[:, c:c + STEP].astype(BF16), kv_step(slot, 1, c),
                                   (((1,), (1,)), ((), ())), preferred_element_type=F32)
            stream.more(pace)
        return acc

    def project(p, acc, denom):
        n = PAIR * WIDE
        at = p * n if isinstance(p, int) else pl.multiple_of(p * n, n)
        return _dot(jnp.where(own, acc / denom, 0.0).astype(BF16), _narrow(wo_v[pl.ds(at, n), :]))

    def attend(p, stream, pace):
        slot = p % NSLOT
        _wait_all(kv_part(slot, 0), sem_kv.at[slot, 0])
        denom = softmax(p, slot, stream, pace)
        stream.more(pace)
        _wait_all(kv_part(slot, 1), sem_kv.at[slot, 1])
        acc = add_values(jnp.zeros((SUB, PAIR), F32), slot, 0, window, stream, pace)
        att_s[...] += project(p, acc, denom)

    def body(p, carry):
        stream = _Stream(pair_copies(p + 1, (p + 1) % NSLOT) + pair_copies(p + 2, (p + 2) % NSLOT)[:2 * lead],
                         (LOOK, lead))
        attend(p, stream, 4)
        stream.upto(per_pair + LOOK)
        return carry

    last = NPAIR - 1
    lax.fori_loop(0, last - 1, body, 0)

    slot = last % NSLOT
    v_parts = list(zip((0,) + V_LAST_PARTS, V_LAST_PARTS))
    w2_parts = list(zip((0,) + W2_PARTS, W2_PARTS))
    w2_q = _view(w2_v, 4)
    w2_copies = [_chain(_sweeps(w2_hbm, w2_q, SUB * (f1 - f0), W2_COPY if f1 < W2_PARTS[-1] else W2_END_COPY,
                                ("w2", i), sem_w2.at[i], (0, SUB * f0), (0, SUB * f0)))
                 for i, (f0, f1) in enumerate(w2_parts)]
    tail = _Stream(
        (kv_copies(last, slot, 0, KV_COPY, "k", sem_kv.at[slot, 0])
         + [cp for i, part in enumerate(v_parts)
            for cp in kv_copies(last, slot, 1, V_LAST_COPY, ("v", i), sem_v.at[i], part)]
         + [cp for part in w2_copies[:-1] for cp in part]),
        (LOOK, lead), w2_copies[-1])
    attend(last - 1, tail, 2)
    tail.wait("k", kv_part(slot, 0), sem_kv.at[slot, 0])
    denom = softmax(last, slot, tail, 2)
    acc = jnp.zeros((SUB, PAIR), F32)
    for i, (c0, c1) in enumerate(v_parts):
        tail.wait(("v", i), kv_part(slot, 1, c0, c1), sem_v.at[i])
        acc = add_values(acc, slot, c0, c1, tail, 2)
    att = att_s[...] + project(last, acc, denom)

    att = jnp.broadcast_to(jnp.sum(att, axis=0, keepdims=True), (SUB, D))
    x1 = x0 + mod(2) * att
    h2 = (_layernorm(x1) * (1.0 + mod(4)) + mod(3)).astype(BF16)
    b1 = b1_v[...].astype(F32)
    acts = []
    for i in range(0, F // LANE, 2):
        u = _dot(h2, _columns(_view(w1_v, D // SUB), SUB * i, 2))
        for j in range(2):
            acts.append(_mish(u[:, j * LANE:(j + 1) * LANE] + jnp.broadcast_to(b1[i + j:i + j + 1], (SUB, LANE))))
    act = jnp.concatenate(acts, axis=1)
    quarter, mxu_rows = F // 4, W2_PARTS[0] // WIDE * SUB
    for i in range(F // LANE):
        if (i + 1) * LANE - i * LANE // quarter * quarter > mxu_rows:
            act_s[i * LANE:(i + 1) * LANE, :] = jnp.broadcast_to(
                acts[i][0:1].astype(BF16).astype(F32), (LANE, LANE)).T
    for i, (f0, f1) in enumerate(w2_parts):
        tail.wait(("w2", i), w2_q.at[:, pl.ds(SUB * f0, SUB * (f1 - f0))], sem_w2.at[i])
        if i == 0:
            a = jnp.concatenate([act[:, k:k + mxu_rows] for k in range(0, F, quarter)], axis=1).astype(BF16)
            y = _dot(a, _narrow(w2_q[:, :SUB * f1, :]))
            once = lax.broadcasted_iota(jnp.int32, (SUB, LANE), 0) == 0
            ys = [jnp.where(once, y[:, c:c + LANE], 0.0) for c in range(0, D, LANE)]
            continue
        for f in range(f0, f1, 2):
            for s in range(4):
                w = w2_q[s, SUB * f:SUB * (f + 2), :].astype(F32)
                for j in range(2):
                    r, c = divmod(f + j, WIDE)
                    k = s * quarter + SUB * r
                    ys[c] += w[SUB * j:SUB * (j + 1)] * act_s[k:k + SUB, :]
    y = jnp.concatenate([jnp.sum(v, axis=0, keepdims=True) for v in ys], axis=1)
    o_ref[...] = (x1[0:1] + mod(5)[0:1] * y).astype(o_ref.dtype)


@jax.jit
def pallas_adaLN_cond__sliding_block_cached__dense_activation_mish__decode_kernel(
    A_x: jax.Array,
    A_k_cache: jax.Array,
    A_v_cache: jax.Array,
    A_wq: jax.Array,
    A_wo: jax.Array,
    B_x: jax.Array,
    B_w1: jax.Array,
    B_b1: jax.Array,
    B_w2: jax.Array,
    c: jax.Array,
    w_mod: jax.Array,
):
    del B_x
    sk = A_k_cache.shape[2]
    window = min(4096, max(256, sk // 4))
    kt = _tiles(jnp.swapaxes(A_k_cache, 2, 3).reshape(H * DH, sk), H * DH // SUB)
    vt = _tiles(jnp.swapaxes(A_v_cache, 2, 3).reshape(H * DH, sk), H * DH // SUB)
    wq, wo, w1, w2, wmod = (_tiles(w, sum(how[0])) for w, how in (
        (A_wq, WQ_COPY), (A_wo, WO_COPY), (B_w1, W1_COPY), (B_w2, W2_COPY), (w_mod, WMOD_COPY)))
    hbm = pl.BlockSpec(memory_space=pltpu.HBM)
    values = 2 * NSLOT * PAIR * window + (2 * H * DH + 6 * D + 2 * F) * D
    out = pl.pallas_call(
        functools.partial(_kernel, window=window),
        out_shape=jax.ShapeDtypeStruct((1, D), A_x.dtype),
        in_specs=[hbm] * 10,
        out_specs=pl.BlockSpec(memory_space=pltpu.VMEM),
        scratch_shapes=[
            pltpu.VMEM((values // LANE, LANE), BF16),
            pltpu.VMEM((1, D), BF16),
            pltpu.VMEM((1, D), BF16),
            pltpu.VMEM((F // LANE, LANE), BF16),
            pltpu.VMEM((NPAIR, SUB, PAIR), F32),
            pltpu.VMEM((SUB, window), F32),
            pltpu.VMEM((SUB, D), F32),
            pltpu.VMEM((SUB, 6 * D), F32),
            pltpu.VMEM((F, LANE), F32),
            pltpu.SemaphoreType.DMA((7,)),
            pltpu.SemaphoreType.DMA((NSLOT, 2)),
            pltpu.SemaphoreType.DMA((len(V_LAST_PARTS),)),
            pltpu.SemaphoreType.DMA((len(W2_PARTS),)),
        ],
        compiler_params=pltpu.CompilerParams(
            vmem_limit_bytes=64 * 2**20,
            disable_semaphore_checks=True,
        ),
        name="adaln_attn_mlp_decode",
    )(A_x.reshape(1, D), kt, vt, wq, wo, w1, B_b1.reshape(F // LANE, LANE), w2, c, wmod)
    return out.reshape(A_x.shape)
```

```python
import functools

import jax
import jax.numpy as jnp
from jax import lax
import jax.experimental.pallas as pl
import jax.experimental.pallas.tpu as pltpu

D = 640
H = 32
DH = 192
F = 1536
PAIR = 2 * DH
NPAIR = H // 2
SUB, LANE = 8, 128
WIDE = D // LANE
F32 = jnp.float32
BF16 = jnp.bfloat16

NSLOT = 3
SKEW = 25
LOOK = 22
KV_COPY = (4,) * 6, 4
WQ_COPY = WO_COPY = (5,) * 3, 4
WMOD_COPY = (2,) * 5, 8
W1_COPY = (2,) * 2, 8
W2_COPY = (1,) * 4, 16
W2_END_COPY = (1,) * 4, 2
PLACE = 2048
W2_END = 224
V_LAST_PARTS = (2048, 3072, 4096)
W2_PARTS = (160, 208, 224, 236, 240)
STEP = 512


def _layernorm(x, eps=1e-5):
    m = jnp.mean(x, axis=-1, keepdims=True)
    d = x - m
    v = jnp.mean(d * d, axis=-1, keepdims=True)
    return d / jnp.sqrt(v + eps)


def _mish(u):
    softplus = jnp.log1p(jnp.exp(-jnp.abs(u))) + jnp.where(u > 0, u, 0.0)
    return u * jnp.tanh(softplus)


def _dot(a, b):
    return jnp.dot(a, b, preferred_element_type=F32)


def _tiles(w, places):
    r, c = w.shape
    return w.reshape(r // SUB, SUB, c // LANE, LANE).transpose(0, 2, 1, 3).reshape(places, -1, LANE)


def _matrix(tiles, width):
    n = width // LANE
    w = tiles.reshape(-1, 2 * SUB * n, LANE)
    cols = [jnp.concatenate([w[:, SUB * c:SUB * (c + 1)], w[:, SUB * (c + n):SUB * (c + n + 1)]], axis=1)
            for c in range(n)]
    return jnp.concatenate([c.reshape(-1, LANE) for c in cols], axis=1)


def _sweeps(src, dst, rows, how, tag, sem, src_at=(0, 0), dst_at=(0, 0)):
    places, tiles = how
    out = []
    for t in range(0, rows, SUB * tiles):
        w = min(SUB * tiles, rows - t)
        s, sweep = 0, []
        for n in places:
            sweep.append((tag, functools.partial(
                pltpu.make_async_copy, src.at[pl.ds(src_at[0] + s, n), pl.ds(src_at[1] + t, w)],
                dst.at[pl.ds(dst_at[0] + s, n), pl.ds(dst_at[1] + t, w)], sem)))
            s += n
        out.append(sweep)
    return out


def _chain(*lists):
    keyed = [((i + 0.5) / len(l), k, x) for k, l in enumerate(lists) for i, x in enumerate(l)]
    return [cp for _, _, sweep in sorted(keyed, key=lambda t: t[:2]) for cp in sweep]


class _Stream:
    def __init__(self, copies, started=(0, 0), end=()):
        self.queue = (copies[0::2], copies[1::2] + list(end))
        self.last = {tag: i // 2 for i, (tag, _) in enumerate(copies)}
        self.started = list(started)

    def start(self, q, n=1):
        for _, copy in self.queue[q][self.started[q]:self.started[q] + n]:
            copy().start(priority=q)
            self.started[q] += 1

    def more(self, n):
        for _ in range(n):
            self.start(1)
            self.start(0)

    def upto(self, n):
        self.more(n - self.started[0])

    def wait(self, tag, ref, sem):
        self.upto(self.last.get(tag, len(self.queue[1])) + 1 + LOOK)
        assert all(t != tag for q in range(2) for t, _ in self.queue[q][self.started[q]:])
        _wait_all(ref, sem)


def _wait_all(ref, sem):
    pltpu.make_async_copy(ref, ref, sem).wait()


def _kernel(x_hbm, k_hbm, v_hbm, wq_hbm, wo_hbm, w1_hbm, b1_hbm, w2_hbm, c_hbm, wmod_hbm, o_ref,
            buf, x_v, c_v, b1_v, q_s, s_s, att_s, mod_s, act_s, sem_w, sem_kv, sem_v, sem_w2, *, window):
    rows = window // LANE * SUB
    kv_v, regions, n = buf.at[pl.ds(0, PAIR // SUB)], [], PAIR // SUB
    for src in (wq_hbm, wo_hbm, wmod_hbm, w1_hbm, w2_hbm):
        regions.append(buf.at[pl.ds(n, src.shape[0]), pl.ds(0, src.shape[1])])
        n += src.shape[0]
    wq_v, wo_v, wmod_v, w1_v, w2_v = regions

    def kv_at(slot, j):
        at = (2 * slot + j) * rows
        return at if isinstance(at, int) else pl.multiple_of(at, rows)

    def kv_copies(p, slot, j, tag, sem, part=(0, window)):
        src = (k_hbm, v_hbm)[j]
        t0, t1 = (c // LANE * SUB for c in part)
        return [cp for r in range(0, PAIR // SUB, sum(KV_COPY[0]))
                for cp in _chain(_sweeps(src, kv_v, t1 - t0, KV_COPY, tag, sem,
                                         (p * (PAIR // SUB) + r, src.shape[1] - rows + t0), (r, kv_at(slot, j) + t0)))]

    def pair_copies(p, slot):
        return [cp for j in range(2) for cp in kv_copies(p, slot, j, "kv", sem_kv.at[slot, j])]

    def weights(src, dst, how, i):
        return _sweeps(src, dst, src.shape[1], how, i, sem_w.at[i])

    def times(a, w_v, width, stream, pace):
        n = w_v.shape[0] // WIDE
        out = 0.0
        for i in range(WIDE):
            out += _dot(a[:, i * LANE:(i + 1) * LANE], _matrix(w_v[pl.ds(n * i, n)], width))
            stream.more(pace)
        return out

    s_c, s_x, s_b1, s_wmod, s_wq, s_wo, s_w1 = range(7)
    small = [functools.partial(pltpu.make_async_copy, s, d, sem_w.at[i])
             for i, s, d in ((s_c, c_hbm, c_v), (s_x, x_hbm, x_v), (s_b1, b1_hbm, b1_v))]
    per_pair = len(pair_copies(0, 0)) // 2
    lead = LOOK + SKEW
    assert 2 * lead <= per_pair

    head = _Stream(_chain(weights(wmod_hbm, wmod_v, WMOD_COPY, s_wmod))
                   + _chain(weights(wq_hbm, wq_v, WQ_COPY, s_wq))
                   + _chain(weights(wo_hbm, wo_v, WO_COPY, s_wo), weights(w1_hbm, w1_v, W1_COPY, s_w1))
                   + pair_copies(0, 0) + pair_copies(1, 1)[:2 * lead])
    head.start(0)
    head.start(1, SKEW + 1)
    for cp in small:
        cp().start()
    head.wait(s_wmod, wmod_v, sem_w.at[s_wmod])
    for cp in small:
        cp().wait()
    cf = c_v[...].astype(F32)
    silu_c = jnp.broadcast_to(cf * jax.nn.sigmoid(cf), (SUB, D)).astype(BF16)
    mod_s[...] = times(silu_c, wmod_v, 6 * D, head, 5)

    def mod(i):
        return mod_s[:, i * D:(i + 1) * D]

    x0 = jnp.broadcast_to(x_v[...].astype(F32), (SUB, D))
    h = (_layernorm(x0) * (1.0 + mod(1)) + mod(0)).astype(BF16)
    head.wait(s_wq, wq_v, sem_w.at[s_wq])
    row = lax.broadcasted_iota(jnp.int32, (SUB, PAIR), 0)
    col = lax.broadcasted_iota(jnp.int32, (SUB, PAIR), 1)
    own = jnp.logical_or(jnp.logical_and(row == 0, col < DH), jnp.logical_and(row == 1, col >= DH))
    q = times(h, wq_v, H * DH, head, 8)
    for p in range(NPAIR):
        q_s[p] = jnp.where(own, q[:, p * PAIR:(p + 1) * PAIR], 0.0)
    att_s[...] = jnp.zeros(att_s.shape, F32)
    head.upto(len(head.queue[0]) - SKEW)
    _wait_all(wo_v, sem_w.at[s_wo])
    _wait_all(w1_v, sem_w.at[s_w1])

    def kv_part(slot, j, c0=0, c1=window):
        return kv_v.at[:, pl.ds(kv_at(slot, j) + c0 // LANE * SUB, (c1 - c0) // LANE * SUB)]

    def kv_step(slot, j, c):
        return _matrix(kv_part(slot, j, c, c + STEP)[...], STEP)

    def softmax(p, slot, stream, pace):
        q = q_s[p].astype(BF16)
        for c in range(0, window, STEP):
            s_s[:, c:c + STEP] = _dot(q, kv_step(slot, 0, c)) * DH ** -0.5
            stream.more(pace)
        s = s_s[...]
        e = jnp.exp(s - jnp.max(s, axis=-1, keepdims=True))
        s_s[...] = e
        return jnp.sum(e, axis=-1, keepdims=True)

    def add_values(acc, slot, c0, c1, stream, pace):
        for c in range(c0, c1, STEP):
            acc += lax.dot_general(s_s[:, c:c + STEP].astype(BF16), kv_step(slot, 1, c),
                                   (((1,), (1,)), ((), ())), preferred_element_type=F32)
            stream.more(pace)
        return acc

    def project(p, acc, denom):
        n, per = PAIR * WIDE // LANE, wo_v.shape[1] // LANE
        tiles = []
        for i in range(n):
            at = (p * n + i) % per * LANE
            tiles.append(wo_v[(p * n + i) // per, pl.ds(at if isinstance(p, int) else pl.multiple_of(at, LANE), LANE)])
        return _dot(jnp.where(own, acc / denom, 0.0).astype(BF16), _matrix(jnp.concatenate(tiles, axis=0), D))

    def attend(p, stream, pace):
        slot = p % NSLOT
        _wait_all(kv_part(slot, 0), sem_kv.at[slot, 0])
        denom = softmax(p, slot, stream, pace)
        stream.more(pace)
        _wait_all(kv_part(slot, 1), sem_kv.at[slot, 1])
        acc = add_values(jnp.zeros((SUB, PAIR), F32), slot, 0, window, stream, pace)
        att_s[...] += project(p, acc, denom)

    def body(p, carry):
        stream = _Stream(pair_copies(p + 1, (p + 1) % NSLOT) + pair_copies(p + 2, (p + 2) % NSLOT)[:2 * lead],
                         (LOOK, lead))
        attend(p, stream, 4)
        stream.upto(per_pair + LOOK)
        return carry

    last = NPAIR - 1
    lax.fori_loop(0, last - 1, body, 0)

    slot = last % NSLOT
    v_parts = list(zip((0,) + V_LAST_PARTS, V_LAST_PARTS))
    w2_parts = list(zip((0,) + W2_PARTS, W2_PARTS))
    w2_copies = [_chain(_sweeps(w2_hbm, w2_v, SUB * (f1 - f0), W2_COPY if f1 <= W2_END else W2_END_COPY,
                                ("w2", i), sem_w2.at[i], (0, SUB * f0), (0, SUB * f0)))
                 for i, (f0, f1) in enumerate(w2_parts)]
    big = W2_PARTS.index(W2_END) + 1
    tail = _Stream(
        (kv_copies(last, slot, 0, "k", sem_kv.at[slot, 0])
         + [cp for i, part in enumerate(v_parts)
            for cp in kv_copies(last, slot, 1, ("v", i), sem_v.at[i], part)]
         + [cp for part in w2_copies[:big] for cp in part]),
        (LOOK, lead), [cp for part in w2_copies[big:] for cp in part])
    attend(last - 1, tail, 2)
    tail.wait("k", kv_part(slot, 0), sem_kv.at[slot, 0])
    denom = softmax(last, slot, tail, 2)
    acc = jnp.zeros((SUB, PAIR), F32)
    for i, (c0, c1) in enumerate(v_parts):
        tail.wait(("v", i), kv_part(slot, 1, c0, c1), sem_v.at[i])
        acc = add_values(acc, slot, c0, c1, tail, 2)
    att = att_s[...] + project(last, acc, denom)

    att = jnp.broadcast_to(jnp.sum(att, axis=0, keepdims=True), (SUB, D))
    x1 = x0 + mod(2) * att
    h2 = (_layernorm(x1) * (1.0 + mod(4)) + mod(3)).astype(BF16)
    b1 = b1_v[...].astype(F32)
    u = _dot(h2, _matrix(w1_v[...], F))
    acts = [_mish(u[:, i * LANE:(i + 1) * LANE] + jnp.broadcast_to(b1[i:i + 1], (SUB, LANE)))
            for i in range(F // LANE)]
    act = jnp.concatenate(acts, axis=1)
    quarter, mxu_rows = F // 4, W2_PARTS[0] // WIDE * SUB
    for i in range(F // LANE):
        if (i + 1) * LANE - i * LANE // quarter * quarter > mxu_rows:
            act_s[i * LANE:(i + 1) * LANE, :] = jnp.broadcast_to(
                acts[i][0:1].astype(BF16).astype(F32), (LANE, LANE)).T
    for i, (f0, f1) in enumerate(w2_parts):
        tail.wait(("w2", i), w2_v.at[:, pl.ds(SUB * f0, SUB * (f1 - f0))], sem_w2.at[i])
        if i == 0:
            a = jnp.concatenate([act[:, k:k + mxu_rows] for k in range(0, F, quarter)], axis=1).astype(BF16)
            y = _dot(a, _matrix(w2_v[:, :SUB * f1, :], D))
            once = lax.broadcasted_iota(jnp.int32, (SUB, LANE), 0) == 0
            ys = [jnp.where(once, y[:, c:c + LANE], 0.0) for c in range(0, D, LANE)]
            continue
        for f in range(f0, f1, 2):
            for s in range(4):
                w = w2_v[s, SUB * f:SUB * (f + 2), :].astype(F32)
                for j in range(2):
                    r, c = divmod(f + j, WIDE)
                    k = s * quarter + SUB * r
                    ys[c] += w[SUB * j:SUB * (j + 1)] * act_s[k:k + SUB, :]
    y = jnp.concatenate([jnp.sum(v, axis=0, keepdims=True) for v in ys], axis=1)
    o_ref[...] = (x1[0:1] + mod(5)[0:1] * y).astype(o_ref.dtype)


@jax.jit
def pallas_adaLN_cond__sliding_block_cached__dense_activation_mish__decode_kernel(
    A_x: jax.Array,
    A_k_cache: jax.Array,
    A_v_cache: jax.Array,
    A_wq: jax.Array,
    A_wo: jax.Array,
    B_x: jax.Array,
    B_w1: jax.Array,
    B_b1: jax.Array,
    B_w2: jax.Array,
    c: jax.Array,
    w_mod: jax.Array,
):
    del B_x
    sk = A_k_cache.shape[2]
    window = min(4096, max(256, sk // 4))
    kt = _tiles(jnp.swapaxes(A_k_cache, 2, 3).reshape(H * DH, sk), H * DH // SUB)
    vt = _tiles(jnp.swapaxes(A_v_cache, 2, 3).reshape(H * DH, sk), H * DH // SUB)
    wq, wo, w1, w2, wmod = weights = [_tiles(w, sum(how[0])) for w, how in (
        (A_wq, WQ_COPY), (A_wo, WO_COPY), (B_w1, W1_COPY), (B_w2, W2_COPY), (w_mod, WMOD_COPY))]
    hbm = pl.BlockSpec(memory_space=pltpu.HBM)
    places = PAIR // SUB + sum(w.shape[0] for w in weights)
    out = pl.pallas_call(
        functools.partial(_kernel, window=window),
        out_shape=jax.ShapeDtypeStruct((1, D), A_x.dtype),
        in_specs=[hbm] * 10,
        out_specs=pl.BlockSpec(memory_space=pltpu.VMEM),
        scratch_shapes=[
            pltpu.VMEM((places, PLACE, LANE), BF16),
            pltpu.VMEM((1, D), BF16),
            pltpu.VMEM((1, D), BF16),
            pltpu.VMEM((F // LANE, LANE), BF16),
            pltpu.VMEM((NPAIR, SUB, PAIR), F32),
            pltpu.VMEM((SUB, window), F32),
            pltpu.VMEM((SUB, D), F32),
            pltpu.VMEM((SUB, 6 * D), F32),
            pltpu.VMEM((F, LANE), F32),
            pltpu.SemaphoreType.DMA((7,)),
            pltpu.SemaphoreType.DMA((NSLOT, 2)),
            pltpu.SemaphoreType.DMA((len(V_LAST_PARTS),)),
            pltpu.SemaphoreType.DMA((len(W2_PARTS),)),
        ],
        compiler_params=pltpu.CompilerParams(
            vmem_limit_bytes=64 * 2**20,
            disable_semaphore_checks=True,
        ),
        name="adaln_attn_mlp_decode",
    )(A_x.reshape(1, D), kt, vt, wq, wo, w1, B_b1.reshape(F // LANE, LANE), w2, c, wmod)
    return out.reshape(A_x.shape)
```

```python
import functools

import jax
import jax.numpy as jnp
from jax import lax
import jax.experimental.pallas as pl
import jax.experimental.pallas.tpu as pltpu

D = 640
H = 32
DH = 192
F = 1536
PAIR = 2 * DH
NPAIR = H // 2
SUB, LANE = 8, 128
WIDE = D // LANE
F32 = jnp.float32
BF16 = jnp.bfloat16

NSLOT = 3
SKEW = 25
LOOK = 18
KV_COPY = (4,) * 6, 4
WQ_COPY = WO_COPY = (2, 4, 4, 5), 4
WMOD_COPY = (2,) * 5, 8
W1_COPY = (2,) * 2, 8
W2_COPY = (2,) * 2, 8
W2_END_COPY = (1,) * 4, 2
PLACE = 2048
W2_END = 228
V_LAST_PARTS = (3072, 4096)
W2_PARTS = (160, 208, 228, 234, 238, 240)
STEP = 512


def _layernorm(x, eps=1e-5):
    m = jnp.mean(x, axis=-1, keepdims=True)
    d = x - m
    v = jnp.mean(d * d, axis=-1, keepdims=True)
    return d / jnp.sqrt(v + eps)


def _mish(u):
    softplus = jnp.log1p(jnp.exp(-jnp.abs(u))) + jnp.where(u > 0, u, 0.0)
    return u * jnp.tanh(softplus)


def _dot(a, b):
    return jnp.dot(a, b, preferred_element_type=F32)


def _tiles(w, places):
    r, c = w.shape
    return w.reshape(r // SUB, SUB, c // LANE, LANE).transpose(0, 2, 1, 3).reshape(places, -1, LANE)


def _matrix(tiles, width):
    n = width // LANE
    w = tiles.reshape(-1, 2 * SUB * n, LANE)
    cols = [jnp.concatenate([w[:, SUB * c:SUB * (c + 1)], w[:, SUB * (c + n):SUB * (c + n + 1)]], axis=1)
            for c in range(n)]
    return jnp.concatenate([c.reshape(-1, LANE) for c in cols], axis=1)


def _sweeps(src, dst, rows, how, tag, sem, src_at=(0, 0), dst_at=(0, 0)):
    places, tiles = how
    out = []
    for t in range(0, rows, SUB * tiles):
        w = min(SUB * tiles, rows - t)
        s, sweep = 0, []
        for n in places:
            sweep.append((tag, functools.partial(
                pltpu.make_async_copy, src.at[pl.ds(src_at[0] + s, n), pl.ds(src_at[1] + t, w)],
                dst.at[pl.ds(dst_at[0] + s, n), pl.ds(dst_at[1] + t, w)], sem)))
            s += n
        out.append(sweep)
    return out


def _chain(*lists):
    keyed = [((i + 0.5) / len(l), k, x) for k, l in enumerate(lists) for i, x in enumerate(l)]
    return [cp for _, _, sweep in sorted(keyed, key=lambda t: t[:2]) for cp in sweep]


class _Stream:
    def __init__(self, copies, started=(0, 0), end=()):
        self.queue = (copies[0::2], copies[1::2] + list(end))
        self.last = {tag: i // 2 for i, (tag, _) in enumerate(copies)}
        self.started = list(started)

    def start(self, q, n=1):
        for _, copy in self.queue[q][self.started[q]:self.started[q] + n]:
            copy().start(priority=q)
            self.started[q] += 1

    def more(self, n):
        for _ in range(n):
            self.start(1)
            self.start(0)

    def upto(self, n):
        self.more(n - self.started[0])

    def wait(self, tag, ref, sem):
        self.upto(self.last.get(tag, len(self.queue[1])) + 1 + LOOK)
        assert all(t != tag for q in range(2) for t, _ in self.queue[q][self.started[q]:])
        _wait_all(ref, sem)


def _wait_all(ref, sem):
    pltpu.make_async_copy(ref, ref, sem).wait()


def _kernel(x_hbm, k_hbm, v_hbm, wq_hbm, wo_hbm, w1_hbm, b1_hbm, w2_hbm, c_hbm, wmod_hbm, o_ref,
            buf, x_v, c_v, b1_v, q_s, s_s, att_s, mod_s, act_s, sem_w, sem_kv, sem_v, sem_w2, *, window):
    rows = window // LANE * SUB
    kv_v, regions, n = buf.at[pl.ds(0, PAIR // SUB)], [], PAIR // SUB
    for src in (wq_hbm, wo_hbm, wmod_hbm, w1_hbm, w2_hbm):
        regions.append(buf.at[pl.ds(n, src.shape[0]), pl.ds(0, src.shape[1])])
        n += src.shape[0]
    wq_v, wo_v, wmod_v, w1_v, w2_v = regions

    def kv_at(slot, j):
        at = (2 * slot + j) * rows
        return at if isinstance(at, int) else pl.multiple_of(at, rows)

    def kv_copies(p, slot, j, tag, sem, part=(0, window)):
        src = (k_hbm, v_hbm)[j]
        t0, t1 = (c // LANE * SUB for c in part)
        first, second = (_sweeps(src, kv_v, t1 - t0, KV_COPY, tag, sem,
                                 (p * (PAIR // SUB) + r, src.shape[1] - rows + t0), (r, kv_at(slot, j) + t0))
                         for r in (0, DH // SUB))
        return _chain(first + second[::-1])

    def pair_copies(p, slot):
        return [cp for j in range(2) for cp in kv_copies(p, slot, j, "kv", sem_kv.at[slot, j])]

    def weights(src, dst, how, i):
        return _sweeps(src, dst, src.shape[1], how, i, sem_w.at[i])

    def times(a, w_v, width, stream, pace):
        n = w_v.shape[0] // WIDE
        out = 0.0
        for i in range(WIDE):
            out += _dot(a[:, i * LANE:(i + 1) * LANE], _matrix(w_v[pl.ds(n * i, n)], width))
            stream.more(pace)
        return out

    s_c, s_x, s_b1, s_wmod, s_wq, s_wo, s_w1 = range(7)
    small = [functools.partial(pltpu.make_async_copy, s, d, sem_w.at[i])
             for i, s, d in ((s_c, c_hbm, c_v), (s_x, x_hbm, x_v), (s_b1, b1_hbm, b1_v))]
    per_pair = len(pair_copies(0, 0)) // 2
    lead = LOOK + SKEW
    assert 2 * lead <= per_pair

    head = _Stream(_chain(weights(wmod_hbm, wmod_v, WMOD_COPY, s_wmod))
                   + _chain(weights(wq_hbm, wq_v, WQ_COPY, s_wq))
                   + _chain(weights(wo_hbm, wo_v, WO_COPY, s_wo), weights(w1_hbm, w1_v, W1_COPY, s_w1))
                   + pair_copies(0, 0) + pair_copies(1, 1)[:2 * lead])
    head.start(0)
    head.start(1, SKEW + 1)
    for cp in small:
        cp().start()
    head.wait(s_wmod, wmod_v, sem_w.at[s_wmod])
    for cp in small:
        cp().wait()
    cf = c_v[...].astype(F32)
    silu_c = jnp.broadcast_to(cf * jax.nn.sigmoid(cf), (SUB, D)).astype(BF16)
    mod_s[...] = times(silu_c, wmod_v, 6 * D, head, 5)

    def mod(i):
        return mod_s[:, i * D:(i + 1) * D]

    x0 = jnp.broadcast_to(x_v[...].astype(F32), (SUB, D))
    h = (_layernorm(x0) * (1.0 + mod(1)) + mod(0)).astype(BF16)
    head.wait(s_wq, wq_v, sem_w.at[s_wq])
    row = lax.broadcasted_iota(jnp.int32, (SUB, PAIR), 0)
    col = lax.broadcasted_iota(jnp.int32, (SUB, PAIR), 1)
    own = jnp.logical_or(jnp.logical_and(row == 0, col < DH), jnp.logical_and(row == 1, col >= DH))
    q = times(h, wq_v, H * DH, head, 8)
    for p in range(NPAIR):
        q_s[p] = jnp.where(own, q[:, p * PAIR:(p + 1) * PAIR], 0.0)
    att_s[...] = jnp.zeros(att_s.shape, F32)
    head.upto(len(head.queue[0]) - SKEW)
    _wait_all(wo_v, sem_w.at[s_wo])
    _wait_all(w1_v, sem_w.at[s_w1])

    def kv_part(slot, j, c0=0, c1=window):
        return kv_v.at[:, pl.ds(kv_at(slot, j) + c0 // LANE * SUB, (c1 - c0) // LANE * SUB)]

    def kv_step(slot, j, c):
        return _matrix(kv_part(slot, j, c, c + STEP)[...], STEP)

    def softmax(p, slot, stream, pace):
        q = q_s[p].astype(BF16)
        for c in range(0, window, STEP):
            s_s[:, c:c + STEP] = _dot(q, kv_step(slot, 0, c)) * DH ** -0.5
            stream.more(pace)
        s = s_s[...]
        e = jnp.exp(s - jnp.max(s, axis=-1, keepdims=True))
        s_s[...] = e
        return jnp.sum(e, axis=-1, keepdims=True)

    def add_values(acc, slot, c0, c1, stream, pace):
        for c in range(c0, c1, STEP):
            acc += lax.dot_general(s_s[:, c:c + STEP].astype(BF16), kv_step(slot, 1, c),
                                   (((1,), (1,)), ((), ())), preferred_element_type=F32)
            stream.more(pace)
        return acc

    def project(p, acc, denom):
        n, per = PAIR * WIDE // LANE, wo_v.shape[1] // LANE
        tiles = []
        for i in range(n):
            at = (p * n + i) % per * LANE
            tiles.append(wo_v[(p * n + i) // per, pl.ds(at if isinstance(p, int) else pl.multiple_of(at, LANE), LANE)])
        return _dot(jnp.where(own, acc / denom, 0.0).astype(BF16), _matrix(jnp.concatenate(tiles, axis=0), D))

    def attend(p, stream, pace):
        slot = p % NSLOT
        _wait_all(kv_part(slot, 0), sem_kv.at[slot, 0])
        denom = softmax(p, slot, stream, pace)
        stream.more(pace)
        _wait_all(kv_part(slot, 1), sem_kv.at[slot, 1])
        acc = add_values(jnp.zeros((SUB, PAIR), F32), slot, 0, window, stream, pace)
        att_s[...] += project(p, acc, denom)

    def body(p, carry):
        stream = _Stream(pair_copies(p + 1, (p + 1) % NSLOT) + pair_copies(p + 2, (p + 2) % NSLOT)[:2 * lead],
                         (LOOK, lead))
        attend(p, stream, 4)
        stream.upto(per_pair + LOOK)
        return carry

    last = NPAIR - 1
    lax.fori_loop(0, last - 1, body, 0)

    slot = last % NSLOT
    v_parts = list(zip((0,) + V_LAST_PARTS, V_LAST_PARTS))
    w2_parts = list(zip((0,) + W2_PARTS, W2_PARTS))
    w2_copies = [_chain(_sweeps(w2_hbm, w2_v, SUB * (f1 - f0), W2_COPY if f1 <= W2_END else W2_END_COPY,
                                ("w2", i), sem_w2.at[i], (0, SUB * f0), (0, SUB * f0)))
                 for i, (f0, f1) in enumerate(w2_parts)]
    big = W2_PARTS.index(W2_END) + 1
    tail = _Stream(
        (kv_copies(last, slot, 0, "k", sem_kv.at[slot, 0])
         + [cp for i, part in enumerate(v_parts)
            for cp in kv_copies(last, slot, 1, ("v", i), sem_v.at[i], part)]
         + [cp for part in w2_copies[:big] for cp in part]),
        (LOOK, lead), [cp for part in w2_copies[big:] for cp in part])
    attend(last - 1, tail, 2)
    tail.wait("k", kv_part(slot, 0), sem_kv.at[slot, 0])
    denom = softmax(last, slot, tail, 2)
    acc = jnp.zeros((SUB, PAIR), F32)
    for i, (c0, c1) in enumerate(v_parts):
        tail.wait(("v", i), kv_part(slot, 1, c0, c1), sem_v.at[i])
        if c1 == window:
            tail.upto(len(tail.queue[1]))
        acc = add_values(acc, slot, c0, c1, tail, 2)
    att = att_s[...] + project(last, acc, denom)

    att = jnp.broadcast_to(jnp.sum(att, axis=0, keepdims=True), (SUB, D))
    x1 = x0 + mod(2) * att
    h2 = (_layernorm(x1) * (1.0 + mod(4)) + mod(3)).astype(BF16)
    b1 = b1_v[...].astype(F32)
    u = _dot(h2, _matrix(w1_v[...], F))
    acts = [_mish(u[:, i * LANE:(i + 1) * LANE] + jnp.broadcast_to(b1[i:i + 1], (SUB, LANE)))
            for i in range(F // LANE)]
    act = jnp.concatenate(acts, axis=1)
    quarter, mxu_rows = F // 4, W2_PARTS[0] // WIDE * SUB
    for i in range(F // LANE):
        if (i + 1) * LANE - i * LANE // quarter * quarter > mxu_rows:
            act_s[i * LANE:(i + 1) * LANE, :] = jnp.broadcast_to(
                acts[i][0:1].astype(BF16).astype(F32), (LANE, LANE)).T
    for i, (f0, f1) in enumerate(w2_parts):
        tail.wait(("w2", i), w2_v.at[:, pl.ds(SUB * f0, SUB * (f1 - f0))], sem_w2.at[i])
        if i == 0:
            a = jnp.concatenate([act[:, k:k + mxu_rows] for k in range(0, F, quarter)], axis=1).astype(BF16)
            y = _dot(a, _matrix(w2_v[:, :SUB * f1, :], D))
            once = lax.broadcasted_iota(jnp.int32, (SUB, LANE), 0) == 0
            ys = [jnp.where(once, y[:, c:c + LANE], 0.0) for c in range(0, D, LANE)]
            continue
        for f in range(f0, f1, 2):
            for s in range(4):
                w = w2_v[s, SUB * f:SUB * (f + 2), :].astype(F32)
                for j in range(2):
                    r, c = divmod(f + j, WIDE)
                    k = s * quarter + SUB * r
                    ys[c] += w[SUB * j:SUB * (j + 1)] * act_s[k:k + SUB, :]
    y = jnp.concatenate([jnp.sum(v, axis=0, keepdims=True) for v in ys], axis=1)
    o_ref[...] = (x1[0:1] + mod(5)[0:1] * y).astype(o_ref.dtype)


@jax.jit
def pallas_adaLN_cond__sliding_block_cached__dense_activation_mish__decode_kernel(
    A_x: jax.Array,
    A_k_cache: jax.Array,
    A_v_cache: jax.Array,
    A_wq: jax.Array,
    A_wo: jax.Array,
    B_x: jax.Array,
    B_w1: jax.Array,
    B_b1: jax.Array,
    B_w2: jax.Array,
    c: jax.Array,
    w_mod: jax.Array,
):
    del B_x
    sk = A_k_cache.shape[2]
    window = min(4096, max(256, sk // 4))
    kt = _tiles(jnp.swapaxes(A_k_cache, 2, 3).reshape(H * DH, sk), H * DH // SUB)
    vt = _tiles(jnp.swapaxes(A_v_cache, 2, 3).reshape(H * DH, sk), H * DH // SUB)
    wq, wo, w1, w2, wmod = weights = [_tiles(w, sum(how[0])) for w, how in (
        (A_wq, WQ_COPY), (A_wo, WO_COPY), (B_w1, W1_COPY), (B_w2, W2_COPY), (w_mod, WMOD_COPY))]
    hbm = pl.BlockSpec(memory_space=pltpu.HBM)
    places = PAIR // SUB + sum(w.shape[0] for w in weights)
    out = pl.pallas_call(
        functools.partial(_kernel, window=window),
        out_shape=jax.ShapeDtypeStruct((1, D), A_x.dtype),
        in_specs=[hbm] * 10,
        out_specs=pl.BlockSpec(memory_space=pltpu.VMEM),
        scratch_shapes=[
            pltpu.VMEM((places, PLACE, LANE), BF16),
            pltpu.VMEM((1, D), BF16),
            pltpu.VMEM((1, D), BF16),
            pltpu.VMEM((F // LANE, LANE), BF16),
            pltpu.VMEM((NPAIR, SUB, PAIR), F32),
            pltpu.VMEM((SUB, window), F32),
            pltpu.VMEM((SUB, D), F32),
            pltpu.VMEM((SUB, 6 * D), F32),
            pltpu.VMEM((F, LANE), F32),
            pltpu.SemaphoreType.DMA((7,)),
            pltpu.SemaphoreType.DMA((NSLOT, 2)),
            pltpu.SemaphoreType.DMA((len(V_LAST_PARTS),)),
            pltpu.SemaphoreType.DMA((len(W2_PARTS),)),
        ],
        compiler_params=pltpu.CompilerParams(
            vmem_limit_bytes=64 * 2**20,
            disable_semaphore_checks=True,
        ),
        name="adaln_attn_mlp_decode",
    )(A_x.reshape(1, D), kt, vt, wq, wo, w1, B_b1.reshape(F // LANE, LANE), w2, c, wmod)
    return out.reshape(A_x.shape)
```

```python
import functools

import jax
import jax.numpy as jnp
from jax import lax
import jax.experimental.pallas as pl
import jax.experimental.pallas.tpu as pltpu

D = 640
H = 32
DH = 192
F = 1536
PAIR = 2 * DH
NPAIR = H // 2
SUB, LANE = 8, 128
WIDE = D // LANE
F32 = jnp.float32
BF16 = jnp.bfloat16

NSLOT = 4
SKEW = 25
LOOK = 18
KV_ROWS, KV_TILES = 4, 4
KV_RUN = 8
KV_SHIFT = 4
WQ_COPY = WO_COPY = (2, 4, 4, 5), 4
WMOD_COPY = (2,) * 5, 8
W1_COPY = (2,) * 2, 8
W2_COPY = (2,) * 2, 8
W2_END_COPY = (1,) * 4, 2
PLACE = 2048
W2_END = 228
V_LAST_PARTS = (3072, 4096)
W2_PARTS = (160, 208, 228, 234, 238, 240)
STEP = 512


def _layernorm(x, eps=1e-5):
    m = jnp.mean(x, axis=-1, keepdims=True)
    d = x - m
    v = jnp.mean(d * d, axis=-1, keepdims=True)
    return d / jnp.sqrt(v + eps)


def _mish(u):
    softplus = jnp.log1p(jnp.exp(-jnp.abs(u))) + jnp.where(u > 0, u, 0.0)
    return u * jnp.tanh(softplus)


def _dot(a, b):
    return jnp.dot(a, b, preferred_element_type=F32)


def _tiles(w, places):
    r, c = w.shape
    return w.reshape(r // SUB, SUB, c // LANE, LANE).transpose(0, 2, 1, 3).reshape(places, -1, LANE)


def _matrix(tiles, width):
    n = width // LANE
    w = tiles.reshape(-1, 2 * SUB * n, LANE)
    cols = [jnp.concatenate([w[:, SUB * c:SUB * (c + 1)], w[:, SUB * (c + n):SUB * (c + n + 1)]], axis=1)
            for c in range(n)]
    return jnp.concatenate([c.reshape(-1, LANE) for c in cols], axis=1)


def _copy(src, src_at, dst, dst_at, shape, sem):
    src, dst = (ref.at[pl.ds(at[0], shape[0]), pl.ds(at[1], shape[1])] for ref, at in ((src, src_at), (dst, dst_at)))
    return pltpu.make_async_copy(src, dst, sem)


def _sweeps(src, dst, how, tag, sem, rows=None):
    places, tiles = how
    r0, r1 = rows or (0, src.shape[1])
    return [[(tag, functools.partial(_copy, src, (sum(places[:i]), r), dst, (sum(places[:i]), r),
                                     (n, min(SUB * tiles, r1 - r)), sem)) for i, n in enumerate(places)]
            for r in range(r0, r1, SUB * tiles)]


def _chain(*lists):
    keyed = [((i + 0.5) / len(l), k, x) for k, l in enumerate(lists) for i, x in enumerate(l)]
    return [cp for _, _, sweep in sorted(keyed, key=lambda t: t[:2]) for cp in sweep]


class _Stream:
    def __init__(self, copies, started=(0, 0), end=()):
        self.queue = (copies[0::2], copies[1::2] + list(end))
        self.last = {tag: i // 2 for i, (tag, _) in enumerate(copies)}
        self.started = list(started)

    def start(self, q, n=1):
        for _, copy in self.queue[q][self.started[q]:self.started[q] + n]:
            copy().start(priority=q)
            self.started[q] += 1

    def more(self, n):
        for _ in range(n):
            self.start(1)
            self.start(0)

    def upto(self, n):
        self.more(n - self.started[0])

    def wait(self, tag, ref, sem):
        self.upto(self.last.get(tag, len(self.queue[1])) + 1 + LOOK)
        assert all(t != tag for q in range(2) for t, _ in self.queue[q][self.started[q]:])
        _wait_all(ref, sem)


def _wait_all(ref, sem):
    pltpu.make_async_copy(ref, ref, sem).wait()


def _kernel(x_hbm, k_hbm, v_hbm, wq_hbm, wo_hbm, w1_hbm, b1_hbm, w2_hbm, c_hbm, wmod_hbm, o_ref,
            buf, x_v, c_v, b1_v, q_s, s_s, att_s, mod_s, act_s, sem_w, sem_kv, sem_v, sem_w2, *, window):
    rows = window // LANE * SUB
    kv_v, regions, n = buf.at[pl.ds(0, PAIR // SUB)], [], PAIR // SUB
    for src in (wq_hbm, wo_hbm, wmod_hbm, w1_hbm, w2_hbm):
        regions.append(buf.at[pl.ds(n, src.shape[0]), pl.ds(0, src.shape[1])])
        n += src.shape[0]
    wq_v, wo_v, wmod_v, w1_v, w2_v = regions

    def kv_at(slot, j):
        at = (2 * slot + j) * rows
        return at if isinstance(at, int) else pl.multiple_of(at, rows)

    def kv_copies(p, j, tag, sem=None, part=(0, window), first=KV_SHIFT, end=PAIR // SUB + KV_SHIFT):
        src = (k_hbm, v_hbm)[j]
        starts = [first] + list(range(KV_SHIFT + KV_RUN, end, KV_RUN))
        runs = [range(r0, r1, KV_ROWS) for r0, r1 in zip(starts, starts[1:] + [end])]
        out = []
        for g in range(0, len(runs), 2):
            at = list(range(part[0] // LANE * SUB, part[1] // LANE * SUB, SUB * KV_TILES))
            if (g // 2 + j) % 2:
                at.reverse()
            for both in zip(at[0::2], at[1::2]):
                for run in runs[g:g + 2]:
                    for t in both:
                        for r in run:
                            slot = (p + r // (PAIR // SUB)) % NSLOT
                            out.append((tag, functools.partial(
                                _copy, src, (p * (PAIR // SUB) + r, src.shape[1] - rows + t),
                                kv_v, (r % (PAIR // SUB), kv_at(slot, j) + t), (KV_ROWS, SUB * KV_TILES),
                                sem_kv.at[slot, j] if sem is None else sem)))
        return out

    def pair_copies(p, **kw):
        return kv_copies(p, 0, "kv", **kw) + kv_copies(p, 1, "kv", **kw)

    def weights(src, dst, how, i):
        return _sweeps(src, dst, how, i, sem_w.at[i])

    def times(a, w_v, width, stream, pace):
        n = w_v.shape[0] // WIDE
        out = 0.0
        for i in range(WIDE):
            out += _dot(a[:, i * LANE:(i + 1) * LANE], _matrix(w_v[pl.ds(n * i, n)], width))
            stream.more(pace)
        return out

    s_c, s_x, s_b1, s_wmod, s_wq, s_wo, s_w1 = range(7)
    small = [functools.partial(pltpu.make_async_copy, s, d, sem_w.at[i])
             for i, s, d in ((s_c, c_hbm, c_v), (s_x, x_hbm, x_v), (s_b1, b1_hbm, b1_v))]
    per_pair = len(pair_copies(1)) // 2
    lead = LOOK + SKEW

    head = _Stream(_chain(weights(w1_hbm, w1_v, W1_COPY, s_w1), weights(wmod_hbm, wmod_v, WMOD_COPY, s_wmod))
                   + _chain(weights(wq_hbm, wq_v, WQ_COPY, s_wq)) + _chain(weights(wo_hbm, wo_v, WO_COPY, s_wo))
                   + pair_copies(0, first=0) + pair_copies(1)[:2 * lead])
    head.start(0)
    head.start(1, SKEW + 1)
    for cp in small:
        cp().start()
    head.wait(s_wmod, wmod_v, sem_w.at[s_wmod])
    for cp in small:
        cp().wait()
    cf = c_v[...].astype(F32)
    silu_c = jnp.broadcast_to(cf * jax.nn.sigmoid(cf), (SUB, D)).astype(BF16)
    mod_s[...] = times(silu_c, wmod_v, 6 * D, head, 5)

    def mod(i):
        return mod_s[:, i * D:(i + 1) * D]

    x0 = jnp.broadcast_to(x_v[...].astype(F32), (SUB, D))
    h = (_layernorm(x0) * (1.0 + mod(1)) + mod(0)).astype(BF16)
    head.wait(s_wq, wq_v, sem_w.at[s_wq])
    row = lax.broadcasted_iota(jnp.int32, (SUB, PAIR), 0)
    col = lax.broadcasted_iota(jnp.int32, (SUB, PAIR), 1)
    own = jnp.logical_or(jnp.logical_and(row == 0, col < DH), jnp.logical_and(row == 1, col >= DH))
    q = times(h, wq_v, H * DH, head, 8)
    for p in range(NPAIR):
        q_s[p] = jnp.where(own, q[:, p * PAIR:(p + 1) * PAIR], 0.0)
    att_s[...] = jnp.zeros(att_s.shape, F32)
    head.upto(len(head.queue[0]) - SKEW)
    _wait_all(wo_v, sem_w.at[s_wo])
    _wait_all(w1_v, sem_w.at[s_w1])

    def kv_part(slot, j, c0=0, c1=window):
        return kv_v.at[:, pl.ds(kv_at(slot, j) + c0 // LANE * SUB, (c1 - c0) // LANE * SUB)]

    def kv_step(slot, j, c):
        return _matrix(kv_part(slot, j, c, c + STEP)[...], STEP)

    def softmax(p, slot, stream, pace):
        q = q_s[p].astype(BF16)
        for c in range(0, window, STEP):
            s_s[:, c:c + STEP] = _dot(q, kv_step(slot, 0, c)) * DH ** -0.5
            stream.more(pace)
        s = s_s[...]
        e = jnp.exp(s - jnp.max(s, axis=-1, keepdims=True))
        s_s[...] = e
        return jnp.sum(e, axis=-1, keepdims=True)

    def add_values(acc, slot, c0, c1, stream, pace):
        for c in range(c0, c1, STEP):
            acc += lax.dot_general(s_s[:, c:c + STEP].astype(BF16), kv_step(slot, 1, c),
                                   (((1,), (1,)), ((), ())), preferred_element_type=F32)
            stream.more(pace)
        return acc

    def project(p, acc, denom):
        n, per = PAIR * WIDE // LANE, wo_v.shape[1] // LANE
        tiles = []
        for i in range(n):
            at = (p * n + i) % per * LANE
            tiles.append(wo_v[(p * n + i) // per, pl.ds(at if isinstance(p, int) else pl.multiple_of(at, LANE), LANE)])
        return _dot(jnp.where(own, acc / denom, 0.0).astype(BF16), _matrix(jnp.concatenate(tiles, axis=0), D))

    def attend(p, stream, pace):
        slot = p % NSLOT
        _wait_all(kv_part(slot, 0), sem_kv.at[slot, 0])
        denom = softmax(p, slot, stream, pace)
        stream.more(pace)
        _wait_all(kv_part(slot, 1), sem_kv.at[slot, 1])
        acc = add_values(jnp.zeros((SUB, PAIR), F32), slot, 0, window, stream, pace)
        att_s[...] += project(p, acc, denom)

    def body(p, carry):
        stream = _Stream(pair_copies(p + 1) + pair_copies(p + 2)[:2 * lead], (LOOK, lead))
        attend(p, stream, 4)
        stream.upto(per_pair + LOOK)
        return carry

    last = NPAIR - 1
    lax.fori_loop(0, last - 2, body, 0)

    slot = last % NSLOT
    v_parts = list(zip((0,) + V_LAST_PARTS, V_LAST_PARTS))
    w2_parts = list(zip((0,) + W2_PARTS, W2_PARTS))
    w2_copies = [_chain(_sweeps(w2_hbm, w2_v, W2_COPY if f1 <= W2_END else W2_END_COPY,
                                ("w2", i), sem_w2.at[i], (SUB * f0, SUB * f1)))
                 for i, (f0, f1) in enumerate(w2_parts)]
    big = W2_PARTS.index(W2_END) + 1
    tail = _Stream(
        (pair_copies(last - 1) + kv_copies(last, 0, "k", end=PAIR // SUB)
         + [cp for i, part in enumerate(v_parts)
            for cp in kv_copies(last, 1, ("v", i), sem_v.at[i], part, end=PAIR // SUB)]
         + [cp for part in w2_copies[:big] for cp in part]),
        (LOOK, lead), [cp for part in w2_copies[big:] for cp in part])
    attend(last - 2, tail, 4)
    tail.upto(per_pair + LOOK)
    attend(last - 1, tail, 2)
    tail.wait("k", kv_part(slot, 0), sem_kv.at[slot, 0])
    denom = softmax(last, slot, tail, 2)
    acc = jnp.zeros((SUB, PAIR), F32)
    _wait_all(kv_part(slot, 1).at[pl.ds(0, KV_SHIFT)], sem_kv.at[slot, 1])
    for i, (c0, c1) in enumerate(v_parts):
        tail.wait(("v", i), kv_part(slot, 1, c0, c1).at[pl.ds(KV_SHIFT, PAIR // SUB - KV_SHIFT)], sem_v.at[i])
        if c1 == window:
            tail.upto(len(tail.queue[1]))
        acc = add_values(acc, slot, c0, c1, tail, 2)
    att = att_s[...] + project(last, acc, denom)

    att = jnp.broadcast_to(jnp.sum(att, axis=0, keepdims=True), (SUB, D))
    x1 = x0 + mod(2) * att
    h2 = (_layernorm(x1) * (1.0 + mod(4)) + mod(3)).astype(BF16)
    b1 = b1_v[...].astype(F32)
    u = _dot(h2, _matrix(w1_v[...], F))
    acts = [_mish(u[:, i * LANE:(i + 1) * LANE] + jnp.broadcast_to(b1[i:i + 1], (SUB, LANE)))
            for i in range(F // LANE)]
    act = jnp.concatenate(acts, axis=1)
    quarter, mxu_rows = F // 4, W2_PARTS[0] // WIDE * SUB
    for i in range(F // LANE):
        if (i + 1) * LANE - i * LANE // quarter * quarter > mxu_rows:
            act_s[i * LANE:(i + 1) * LANE, :] = jnp.broadcast_to(
                acts[i][0:1].astype(BF16).astype(F32), (LANE, LANE)).T
    for i, (f0, f1) in enumerate(w2_parts):
        tail.wait(("w2", i), w2_v.at[:, pl.ds(SUB * f0, SUB * (f1 - f0))], sem_w2.at[i])
        if i == 0:
            a = jnp.concatenate([act[:, k:k + mxu_rows] for k in range(0, F, quarter)], axis=1).astype(BF16)
            y = _dot(a, _matrix(w2_v[:, :SUB * f1, :], D))
            once = lax.broadcasted_iota(jnp.int32, (SUB, LANE), 0) == 0
            ys = [jnp.where(once, y[:, c:c + LANE], 0.0) for c in range(0, D, LANE)]
            continue
        for f in range(f0, f1, 2):
            for s in range(4):
                w = w2_v[s, SUB * f:SUB * (f + 2), :].astype(F32)
                for j in range(2):
                    r, c = divmod(f + j, WIDE)
                    k = s * quarter + SUB * r
                    ys[c] += w[SUB * j:SUB * (j + 1)] * act_s[k:k + SUB, :]
    y = jnp.concatenate([jnp.sum(v, axis=0, keepdims=True) for v in ys], axis=1)
    o_ref[...] = (x1[0:1] + mod(5)[0:1] * y).astype(o_ref.dtype)


@jax.jit
def pallas_adaLN_cond__sliding_block_cached__dense_activation_mish__decode_kernel(
    A_x: jax.Array,
    A_k_cache: jax.Array,
    A_v_cache: jax.Array,
    A_wq: jax.Array,
    A_wo: jax.Array,
    B_x: jax.Array,
    B_w1: jax.Array,
    B_b1: jax.Array,
    B_w2: jax.Array,
    c: jax.Array,
    w_mod: jax.Array,
):
    del B_x
    sk = A_k_cache.shape[2]
    window = min(4096, max(256, sk // 4))
    kt = _tiles(jnp.swapaxes(A_k_cache, 2, 3).reshape(H * DH, sk), H * DH // SUB)
    vt = _tiles(jnp.swapaxes(A_v_cache, 2, 3).reshape(H * DH, sk), H * DH // SUB)
    wq, wo, w1, w2, wmod = weights = [_tiles(w, sum(how[0])) for w, how in (
        (A_wq, WQ_COPY), (A_wo, WO_COPY), (B_w1, W1_COPY), (B_w2, W2_COPY), (w_mod, WMOD_COPY))]
    hbm = pl.BlockSpec(memory_space=pltpu.HBM)
    places = PAIR // SUB + sum(w.shape[0] for w in weights)
    out = pl.pallas_call(
        functools.partial(_kernel, window=window),
        out_shape=jax.ShapeDtypeStruct((1, D), A_x.dtype),
        in_specs=[hbm] * 10,
        out_specs=pl.BlockSpec(memory_space=pltpu.VMEM),
        scratch_shapes=[
            pltpu.VMEM((places, PLACE, LANE), BF16),
            pltpu.VMEM((1, D), BF16),
            pltpu.VMEM((1, D), BF16),
            pltpu.VMEM((F // LANE, LANE), BF16),
            pltpu.VMEM((NPAIR, SUB, PAIR), F32),
            pltpu.VMEM((SUB, window), F32),
            pltpu.VMEM((SUB, D), F32),
            pltpu.VMEM((SUB, 6 * D), F32),
            pltpu.VMEM((F, LANE), F32),
            pltpu.SemaphoreType.DMA((7,)),
            pltpu.SemaphoreType.DMA((NSLOT, 2)),
            pltpu.SemaphoreType.DMA((len(V_LAST_PARTS),)),
            pltpu.SemaphoreType.DMA((len(W2_PARTS),)),
        ],
        compiler_params=pltpu.CompilerParams(
            vmem_limit_bytes=64 * 2**20,
            disable_semaphore_checks=True,
        ),
        name="adaln_attn_mlp_decode",
    )(A_x.reshape(1, D), kt, vt, wq, wo, w1, B_b1.reshape(F // LANE, LANE), w2, c, wmod)
    return out.reshape(A_x.shape)
```
